```python
import os as _os
_os.environ.setdefault("JAX_PLATFORMS", "cpu")
import jax
import jax.numpy as jnp

def _softmax(x, axis=-1):
    return jax.nn.softmax(x, axis=axis)
def _gelu(x):
    return jax.nn.gelu(x, approximate=True)
def _silu(x):
    return jax.nn.silu(x)
def _sigmoid(x):
    return jax.nn.sigmoid(x)
def _layernorm(x, axis=-1, eps=1e-5):
    m = jnp.mean(x, axis=axis, keepdims=True)
    v = jnp.var(x, axis=axis, keepdims=True)
    return (x - m) / jnp.sqrt(v + eps)
def _scatter_add(tgt, idx, src, axis=0):
    return tgt.at[idx].add(src)
def _segment_sum(src, seg, n):
    return jax.ops.segment_sum(src, seg, n)
class _Rng:
    def __init__(self, key):
        self._k = key
    def _next(self):
        self._k, sub = jax.random.split(self._k)
        return sub
    def normal(self, shape):
        return jax.random.normal(self._next(), shape, dtype=jnp.bfloat16)
    def randint(self, lo, hi, shape):
        return jax.random.randint(self._next(), shape, lo, hi, dtype=jnp.int32)
    def uniform(self, shape, lo=0.0, hi=1.0):
        return jax.random.uniform(self._next(), shape, jnp.bfloat16, lo, hi)
    def permutation(self, n):
        return jax.random.permutation(self._next(), n)


kernel_name = 'parallel_sum__sliding_block__moe_arch_mod__prompt'

def setup_inputs():
    _rng = _Rng(jax.random.key(int.from_bytes(__import__("os").urandom(4), "little")))
    _w = (lambda a: (lambda t: t.astype(jnp.bfloat16) if jnp.issubdtype(t.dtype, jnp.floating) else t)(jnp.asarray(a)))
    def _A_setup():
        B, S, D = 1, 2048, 512
        return {
            "x": _w((lambda *s: _rng.normal(s) * 0.05)(B, S, D)),
            "wqkv": _w((lambda *s: _rng.normal(s) * 0.05)(D, 3 * D)),
            "wo": _w((lambda *s: _rng.normal(s) * 0.05)(D, D)),
        }
    _A_in = _A_setup()

    def _B_setup():
        B, S, D, F, C = 1, 2048, 512, 1376, 1
        return {
            "x": _w((lambda *s: _rng.normal(s) * 0.05)(B, S, D)),
            "w_r": _w((lambda *s: _rng.normal(s) * 0.05)(D)),
            "w_gate": _w((lambda *s: _rng.normal(s) * 0.05)(D, F)),
            "w_up": _w((lambda *s: _rng.normal(s) * 0.05)(D, F)),
            "w_down": _w((lambda *s: _rng.normal(s) * 0.05)(F, D)),
        }
    _B_in = _B_setup()

    return {
        "A_x": _A_in["x"],
        "A_wqkv": _A_in["wqkv"],
        "A_wo": _A_in["wo"],
        "B_x": _B_in["x"],
        "B_w_r": _B_in["w_r"],
        "B_w_gate": _B_in["w_gate"],
        "B_w_up": _B_in["w_up"],
        "B_w_down": _B_in["w_down"],
    }

def reference(A_x, A_wqkv, A_wo, B_x, B_w_r, B_w_gate, B_w_up, B_w_down):
    def _A_ref(x, wqkv, wo):
        B, S, D = x.shape
        H = 32; Dh = D // H; W = 256
        qkv = (lambda x, *d: x.transpose(*d))((x @ wqkv).reshape(B, S, 3, H, Dh), 2, 0, 3, 1, 4)
        q, k, v = qkv[0], qkv[1], qkv[2]
        scores = jnp.einsum("bhqd,bhkd->bhqk", q, k) * (Dh ** -0.5)
        idx = jnp.arange(S)
        mask = (idx[:, None] - idx[None, :] >= 0) & (idx[:, None] - idx[None, :] < W)
        scores = jnp.where(mask[None, None], scores, -1e9)
        p = _softmax(scores, axis=-1)
        o = jnp.einsum("bhqk,bhkd->bhqd", p, v)
        return (lambda x, *d: x.transpose(*d))(o, 0, 2, 1, 3).reshape(B, S, D) @ wo

    def _B_ref(x, w_r, w_gate, w_up, w_down):
        B, S, D = x.shape
        C = 1
        r = x @ w_r
        idx = jnp.argsort(-r, axis=-1)[:, :C]
        idx_e = jnp.repeat(idx.reshape(B, C, 1), D, axis=2)
        x_sel = jnp.take_along_axis(x, idx_e, axis=1)
        g = _silu(x_sel @ w_gate)
        u = x_sel @ w_up
        y = (g * u) @ w_down
        r_sel = _sigmoid(jnp.take_along_axis(r, idx, axis=1))
        y = y * r_sel.reshape(B, C, 1)
        b_off = (jnp.arange(B) * S).reshape(B, 1)
        flat_idx = (idx + b_off).reshape(B * C)
        zero = (x * 0.0).reshape(B * S, D)
        upd = _scatter_add(zero, flat_idx, y.reshape(B * C, D), axis=0)
        return x + upd.reshape(B, S, D)

    x = A_x
    xn = _layernorm(x, axis=-1)
    return x + _A_ref(xn, A_wqkv, A_wo) + _B_ref(xn, B_w_r, B_w_gate, B_w_up, B_w_down)
```

```python
import functools
import jax
import jax.numpy as jnp
from jax import lax
from jax.experimental import pallas as pl
from jax.experimental.pallas import tpu as pltpu

S, D, H, DH, WIN, F = 2048, 512, 32, 16, 256, 1376
QB = 128
NB = S // QB
HG = 128 // DH
NG = H // HG
KW = WIN + QB
NTILE = KW // 128
PAD = WIN
NEG = -1e30
LOG2E = 1.4426950408889634
F32, BF16 = jnp.float32, jnp.bfloat16
NT = (((1,), (1,)), ((), ()))


def _rb(t):
    return t.astype(BF16).astype(F32)


def _kernel(x_ref, wqkv_ref, wo_ref, wr_ref, wg_ref, wu_ref, wd_ref, o_ref,
            xn_ref, qm_ref, k_ref, v_ref, att_ref, bias_ref,
            s00_ref, s01_ref, s02_ref, s10_ref, s11_ref, s12_ref,
            s20_ref, s21_ref, s22_ref, s30_ref, s31_ref, s32_ref,
            m0_ref, m1_ref, m2_ref, m3_ref, l0_ref, l1_ref, l2_ref, l3_ref,
            p00_ref, p01_ref, p02_ref, p10_ref, p11_ref, p12_ref,
            p20_ref, p21_ref, p22_ref, p30_ref, p31_ref, p32_ref):
    x = x_ref[...].astype(F32)
    mean = jnp.mean(x, axis=1, keepdims=True)
    xc = x - mean
    var = jnp.mean(xc * xc, axis=1, keepdims=True)
    d = _rb(x - _rb(mean))
    den = _rb(jnp.sqrt(_rb(_rb(var) + 1e-5)))
    xn = (d / den).astype(BF16)
    xn_ref[...] = xn

    lane = lax.broadcasted_iota(jnp.int32, (1, 128), 1)
    q = jnp.dot(xn, wqkv_ref[:, 0:D], preferred_element_type=F32) * (DH ** -0.5 * LOG2E)
    for g in range(NG):
        qg = q[:, g * 128:(g + 1) * 128]
        for h in range(HG):
            qh = jnp.where(lane // DH == h, qg, 0.0).astype(BF16)
            qm_ref[:, g, h * QB:(h + 1) * QB, :] = qh.reshape(NB, QB, 128)
    k_ref[0:PAD, :] = jnp.zeros((PAD, D), BF16)
    v_ref[0:PAD, :] = jnp.zeros((PAD, D), BF16)
    k_ref[PAD:, :] = jnp.dot(xn, wqkv_ref[:, D:2 * D], preferred_element_type=F32).astype(BF16)
    v_ref[PAD:, :] = jnp.dot(xn, wqkv_ref[:, 2 * D:3 * D], preferred_element_type=F32).astype(BF16)

    qi = lax.broadcasted_iota(jnp.int32, (QB, KW), 0)
    kj = lax.broadcasted_iota(jnp.int32, (QB, KW), 1)
    band = jnp.logical_and(qi + WIN - kj >= 0, qi + WIN - kj < WIN)
    for kind in range(3):
        ok = jnp.logical_and(band, kj >= WIN - kind * QB)
        bfull = jnp.where(ok, 0.0, NEG)
        for t in range(NTILE):
            bias_ref[kind, t] = bfull[:, t * 128:(t + 1) * 128]

    lane_head = lax.broadcasted_iota(jnp.int32, (QB, 128), 1) // DH
    s_bufs = ((s00_ref, s01_ref, s02_ref), (s10_ref, s11_ref, s12_ref),
              (s20_ref, s21_ref, s22_ref), (s30_ref, s31_ref, s32_ref))
    m_bufs, l_bufs = (m0_ref, m1_ref, m2_ref, m3_ref), (l0_ref, l1_ref, l2_ref, l3_ref)
    p_bufs = ((p00_ref, p01_ref, p02_ref), (p10_ref, p11_ref, p12_ref),
              (p20_ref, p21_ref, p22_ref), (p30_ref, p31_ref, p32_ref))

    def stage_a(b, g, t):
        row0 = pl.multiple_of(b * QB, QB)
        qm = qm_ref[b, g]
        kt = k_ref[pl.ds(row0 + t * 128, 128), g * 128:(g + 1) * 128]
        s = lax.dot_general(qm, kt, NT, preferred_element_type=F32)
        bias = bias_ref[jnp.minimum(b, 2), t]
        s_bufs[g][t][...] = (s.reshape(HG, QB, 128) + bias[None]).reshape(HG * QB, 128)

    def stage_b1(g, h):
        rows = slice(h * QB, (h + 1) * QB)
        mx = jnp.maximum(jnp.maximum(s_bufs[g][0][rows, :], s_bufs[g][1][rows, :]), s_bufs[g][2][rows, :])
        m = jnp.max(mx, axis=-1, keepdims=True)
        m_bufs[g][rows, :] = jnp.broadcast_to(m, (QB, 128))

    def stage_b2(g, h):
        rows = slice(h * QB, (h + 1) * QB)
        m = m_bufs[g][rows, :]
        acc = None
        for t in range(NTILE):
            pb = jnp.exp2(s_bufs[g][t][rows, :] - m).astype(BF16)
            p_bufs[g][t][rows, :] = pb
            pr = pb.astype(F32)
            acc = pr if acc is None else acc + pr
        l = jnp.sum(acc, axis=-1, keepdims=True)
        l_bufs[g][rows, :] = jnp.broadcast_to(l, (QB, 128))

    def stage_c(b, g, t, acc):
        row0 = pl.multiple_of(b * QB, QB)
        vt = v_ref[pl.ds(row0 + t * 128, 128), g * 128:(g + 1) * 128]
        r = jnp.dot(p_bufs[g][t][...], vt, preferred_element_type=F32).reshape(HG, QB, 128)
        o = r[0]
        for h in range(1, HG):
            o = jnp.where(lane_head == h, r[h], o)
        acc = o if acc is None else acc + o
        if t == NTILE - 1:
            lall = l_bufs[g][...].reshape(HG, QB, 128)
            lm = lall[0]
            for h in range(1, HG):
                lm = jnp.where(lane_head == h, lall[h], lm)
            att_ref[pl.ds(row0, QB), g * 128:(g + 1) * 128] = (acc / lm).astype(BF16)
        return acc

    def back(b, g, k):
        return (b, g - k) if g >= k else (b - 1, g - k + NG)

    def step(b, g, do_a, do_b1, do_b2, do_c):
        b1 = back(b, g, 1); b2 = back(b, g, 2); c3 = back(b, g, 3)
        hs1 = ((0, 1, 2), (3, 4, 5), (6, 7))
        hs2 = ((0, 1, 2), (3, 4, 5), (6, 7))
        acc = None
        for t in range(NTILE):
            if do_a:
                stage_a(b, g, t)
            if do_b1:
                for h in hs1[t]:
                    stage_b1(b1[1], h)
            if do_c:
                acc = stage_c(c3[0], c3[1], t, acc)
            if do_b2:
                for h in hs2[t]:
                    stage_b2(b2[1], h)

    def qblock(b, first):
        for g in range(NG):
            step(b, g, True, g >= 1 or not first, g >= 2 or not first, g >= 3 or not first)

    qblock(0, True)

    def loop_body(b, carry):
        qblock(b, False)
        return carry

    lax.fori_loop(1, NB, loop_body, 0)
    step(NB, 0, False, True, True, True)
    step(NB, 1, False, False, True, True)
    step(NB, 2, False, False, False, True)

    xnf = xn_ref[...].astype(F32)
    rsc = _rb(jnp.sum(xnf * wr_ref[...].astype(F32), axis=1, keepdims=True))
    rows = lax.broadcasted_iota(jnp.int32, (S, 1), 0)
    rmax = jnp.max(rsc, axis=0, keepdims=True)
    idx = jnp.min(jnp.where(rsc == rmax, rows, S), axis=0, keepdims=True)
    sel = rows == idx
    xs = jnp.sum(jnp.where(sel, xnf, 0.0), axis=0, keepdims=True).astype(BF16)
    xs8 = jnp.broadcast_to(xs, (8, D))
    gp = _rb(jnp.dot(xs8, wg_ref[...], preferred_element_type=F32))
    up = _rb(jnp.dot(xs8, wu_ref[...], preferred_element_type=F32))
    gact = _rb(gp * _rb(jax.nn.sigmoid(gp)))
    hmid = (gact * up).astype(BF16)
    y = _rb(jnp.dot(hmid, wd_ref[...], preferred_element_type=F32))[0:1, :]
    y = _rb(y * _rb(jax.nn.sigmoid(rmax)))

    att = _rb(jnp.dot(att_ref[...], wo_ref[...], preferred_element_type=F32))
    bres = _rb(xnf + jnp.where(sel, y, 0.0))
    o_ref[...] = (_rb(x + att) + bres).astype(BF16)


@jax.jit
def pallas_parallel_sum__sliding_block__moe_arch_mod__prompt_kernel(
        A_x, A_wqkv, A_wo, B_x, B_w_r, B_w_gate, B_w_up, B_w_down):
    x2 = A_x.reshape(S, D)
    wr = B_w_r.reshape(1, D)
    sc = lambda: pltpu.VMEM((HG * QB, 128), F32)
    pb = lambda: pltpu.VMEM((HG * QB, 128), BF16)
    out = pl.pallas_call(
        _kernel,
        out_shape=jax.ShapeDtypeStruct((S, D), BF16),
        scratch_shapes=[
            pltpu.VMEM((S, D), BF16),
            pltpu.VMEM((NB, NG, HG * QB, 128), BF16),
            pltpu.VMEM((S + PAD, D), BF16),
            pltpu.VMEM((S + PAD, D), BF16),
            pltpu.VMEM((S, D), BF16),
            pltpu.VMEM((3, NTILE, QB, 128), F32),
            sc(), sc(), sc(), sc(), sc(), sc(),
            sc(), sc(), sc(), sc(), sc(), sc(),
            sc(), sc(), sc(), sc(),
            sc(), sc(), sc(), sc(),
            pb(), pb(), pb(), pb(), pb(), pb(),
            pb(), pb(), pb(), pb(), pb(), pb(),
        ],
        compiler_params=pltpu.CompilerParams(vmem_limit_bytes=110 * 1024 * 1024),
    )(x2, A_wqkv, A_wo, wr, B_w_gate, B_w_up, B_w_down)
    return out.reshape(1, S, D)
```

```python
import functools
import jax
import jax.numpy as jnp
from jax import lax
from jax.experimental import pallas as pl
from jax.experimental.pallas import tpu as pltpu

S, D, H, DH, WIN, F = 2048, 512, 32, 16, 256, 1376
QB = 128
NB = S // QB
HG = 128 // DH
NG = H // HG
KW = WIN + QB
NTILE = KW // 128
PAD = WIN
NEG = -1e30
NCH = 4
CH = S // NCH
LOG2E = 1.4426950408889634
F32, BF16 = jnp.float32, jnp.bfloat16
NT = (((1,), (1,)), ((), ()))


def _rb(t):
    return t.astype(BF16).astype(F32)


def _kernel(x_hbm, wqkv_hbm, wo_hbm, wr_ref, wg_hbm, wu_hbm, wd_hbm, o_hbm,
            x_ref, wqkv_ref, wo_ref, wg_ref, wu_ref, wd_ref, o_ref, sems,
            xn_ref, qm_ref, k_ref, v_ref, att_ref, bias_ref,
            s00_ref, s01_ref, s02_ref, s10_ref, s11_ref, s12_ref,
            s20_ref, s21_ref, s22_ref, s30_ref, s31_ref, s32_ref,
            m0_ref, m1_ref, m2_ref, m3_ref, l0_ref, l1_ref, l2_ref, l3_ref,
            p00_ref, p01_ref, p02_ref, p10_ref, p11_ref, p12_ref,
            p20_ref, p21_ref, p22_ref, p30_ref, p31_ref, p32_ref):
    def cp(i, src, dst):
        return pltpu.make_async_copy(src, dst, sems.at[i])

    x_cps = [cp(c, x_hbm.at[pl.ds(c * CH, CH)], x_ref.at[pl.ds(c * CH, CH)]) for c in range(NCH)]
    wq_cp = cp(NCH, wqkv_hbm.at[:, pl.ds(0, D)], wqkv_ref.at[:, pl.ds(0, D)])
    wkv_cp = cp(NCH + 1, wqkv_hbm.at[:, pl.ds(D, 2 * D)], wqkv_ref.at[:, pl.ds(D, 2 * D)])
    late_cps = [cp(NCH + 2 + i, s_, d_) for i, (s_, d_) in enumerate((
        (wo_hbm, wo_ref), (wg_hbm, wg_ref), (wu_hbm, wu_ref), (wd_hbm, wd_ref)))]
    x_cps[0].start()
    wq_cp.start()
    x_cps[0].wait()
    wq_cp.wait()
    for c_ in x_cps[1:] + [wkv_cp] + late_cps:
        c_.start()

    lane = lax.broadcasted_iota(jnp.int32, (1, 128), 1)
    for c in range(NCH):
        if c > 0:
            x_cps[c].wait()
        rows = slice(c * CH, (c + 1) * CH)
        x = x_ref[rows, :].astype(F32)
        mean = jnp.mean(x, axis=1, keepdims=True)
        xc = x - mean
        var = jnp.mean(xc * xc, axis=1, keepdims=True)
        d = _rb(x - _rb(mean))
        den = _rb(jnp.sqrt(_rb(_rb(var) + 1e-5)))
        xn = (d / den).astype(BF16)
        xn_ref[rows, :] = xn
        q = jnp.dot(xn, wqkv_ref[:, 0:D], preferred_element_type=F32) * (DH ** -0.5 * LOG2E)
        blk = slice(c * CH // QB, (c + 1) * CH // QB)
        for g in range(NG):
            qg = q[:, g * 128:(g + 1) * 128]
            for h in range(HG):
                qh = jnp.where(lane // DH == h, qg, 0.0).astype(BF16)
                qm_ref[blk, g, h * QB:(h + 1) * QB, :] = qh.reshape(CH // QB, QB, 128)
    wkv_cp.wait()
    xn = xn_ref[...]
    k_ref[0:PAD, :] = jnp.zeros((PAD, D), BF16)
    v_ref[0:PAD, :] = jnp.zeros((PAD, D), BF16)
    k_ref[PAD:, :] = jnp.dot(xn, wqkv_ref[:, D:2 * D], preferred_element_type=F32).astype(BF16)
    v_ref[PAD:, :] = jnp.dot(xn, wqkv_ref[:, 2 * D:3 * D], preferred_element_type=F32).astype(BF16)

    qi = lax.broadcasted_iota(jnp.int32, (QB, KW), 0)
    kj = lax.broadcasted_iota(jnp.int32, (QB, KW), 1)
    band = jnp.logical_and(qi + WIN - kj >= 0, qi + WIN - kj < WIN)
    for kind in range(3):
        ok = jnp.logical_and(band, kj >= WIN - kind * QB)
        bfull = jnp.where(ok, 0.0, NEG)
        for t in range(NTILE):
            bias_ref[kind, t] = bfull[:, t * 128:(t + 1) * 128]

    lane_head = lax.broadcasted_iota(jnp.int32, (QB, 128), 1) // DH
    s_bufs = ((s00_ref, s01_ref, s02_ref), (s10_ref, s11_ref, s12_ref),
              (s20_ref, s21_ref, s22_ref), (s30_ref, s31_ref, s32_ref))
    m_bufs, l_bufs = (m0_ref, m1_ref, m2_ref, m3_ref), (l0_ref, l1_ref, l2_ref, l3_ref)
    p_bufs = ((p00_ref, p01_ref, p02_ref), (p10_ref, p11_ref, p12_ref),
              (p20_ref, p21_ref, p22_ref), (p30_ref, p31_ref, p32_ref))

    def stage_a(b, g, t):
        row0 = pl.multiple_of(b * QB, QB)
        qm = qm_ref[b, g]
        kt = k_ref[pl.ds(row0 + t * 128, 128), g * 128:(g + 1) * 128]
        s = lax.dot_general(qm, kt, NT, preferred_element_type=F32)
        bias = bias_ref[jnp.minimum(b, 2), t]
        s_bufs[g][t][...] = (s.reshape(HG, QB, 128) + bias[None]).reshape(HG * QB, 128)

    def stage_b1(g, h):
        rows = slice(h * QB, (h + 1) * QB)
        mx = jnp.maximum(jnp.maximum(s_bufs[g][0][rows, :], s_bufs[g][1][rows, :]), s_bufs[g][2][rows, :])
        m = jnp.max(mx, axis=-1, keepdims=True)
        m_bufs[g][rows, :] = jnp.broadcast_to(m, (QB, 128))

    def stage_b2(g, h):
        rows = slice(h * QB, (h + 1) * QB)
        m = m_bufs[g][rows, :]
        acc = None
        for t in range(NTILE):
            pb = jnp.exp2(s_bufs[g][t][rows, :] - m).astype(BF16)
            p_bufs[g][t][rows, :] = pb
            pr = pb.astype(F32)
            acc = pr if acc is None else acc + pr
        l = jnp.sum(acc, axis=-1, keepdims=True)
        l_bufs[g][rows, :] = jnp.broadcast_to(l, (QB, 128))

    def stage_c(b, g, t, acc):
        row0 = pl.multiple_of(b * QB, QB)
        vt = v_ref[pl.ds(row0 + t * 128, 128), g * 128:(g + 1) * 128]
        r = jnp.dot(p_bufs[g][t][...], vt, preferred_element_type=F32).reshape(HG, QB, 128)
        o = r[0]
        for h in range(1, HG):
            o = jnp.where(lane_head == h, r[h], o)
        acc = o if acc is None else acc + o
        if t == NTILE - 1:
            lall = l_bufs[g][...].reshape(HG, QB, 128)
            lm = lall[0]
            for h in range(1, HG):
                lm = jnp.where(lane_head == h, lall[h], lm)
            att_ref[pl.ds(row0, QB), g * 128:(g + 1) * 128] = (acc / lm).astype(BF16)
        return acc

    def back(b, g, k):
        return (b, g - k) if g >= k else (b - 1, g - k + NG)

    def step(b, g, do_a, do_b1, do_b2, do_c):
        b1 = back(b, g, 1); b2 = back(b, g, 2); c3 = back(b, g, 3)
        hs1 = ((0, 1, 2), (3, 4, 5), (6, 7))
        hs2 = ((0, 1, 2), (3, 4, 5), (6, 7))
        acc = None
        for t in range(NTILE):
            if do_a:
                stage_a(b, g, t)
            if do_b1:
                for h in hs1[t]:
                    stage_b1(b1[1], h)
            if do_c:
                acc = stage_c(c3[0], c3[1], t, acc)
            if do_b2:
                for h in hs2[t]:
                    stage_b2(b2[1], h)

    def qblock(b, first):
        for g in range(NG):
            step(b, g, True, g >= 1 or not first, g >= 2 or not first, g >= 3 or not first)

    qblock(0, True)

    def loop_body(b, carry):
        qblock(b, False)
        return carry

    lax.fori_loop(1, NB, loop_body, 0)
    step(NB, 0, False, True, True, True)
    step(NB, 1, False, False, True, True)
    step(NB, 2, False, False, False, True)

    for c_ in late_cps:
        c_.wait()
    xnf = xn_ref[...].astype(F32)
    rsc = _rb(jnp.sum(xnf * wr_ref[...].astype(F32), axis=1, keepdims=True))
    rows = lax.broadcasted_iota(jnp.int32, (S, 1), 0)
    rmax = jnp.max(rsc, axis=0, keepdims=True)
    idx = jnp.min(jnp.where(rsc == rmax, rows, S), axis=0, keepdims=True)
    sel = rows == idx
    xs = jnp.sum(jnp.where(sel, xnf, 0.0), axis=0, keepdims=True).astype(BF16)
    xs8 = jnp.broadcast_to(xs, (8, D))
    gp = _rb(lax.dot_general(xs8, wg_ref[...], NT, preferred_element_type=F32))
    up = _rb(lax.dot_general(xs8, wu_ref[...], NT, preferred_element_type=F32))
    gact = _rb(gp * _rb(jax.nn.sigmoid(gp)))
    hmid = (gact * up).astype(BF16)
    y = _rb(jnp.dot(hmid, wd_ref[...], preferred_element_type=F32))[0:1, :]
    y = _rb(y * _rb(jax.nn.sigmoid(rmax)))

    out_cps = []
    for c in range(NCH):
        rows = slice(c * CH, (c + 1) * CH)
        att = _rb(jnp.dot(att_ref[rows, :], wo_ref[...], preferred_element_type=F32))
        bres = _rb(xnf[rows, :] + jnp.where(sel[rows, :], y, 0.0))
        o_ref[rows, :] = (_rb(x_ref[rows, :].astype(F32) + att) + bres).astype(BF16)
        cp_out = pltpu.make_async_copy(o_ref.at[pl.ds(c * CH, CH)], o_hbm.at[pl.ds(c * CH, CH)],
                                       sems.at[NCH + 6 + c])
        cp_out.start()
        out_cps.append(cp_out)
    for c_ in out_cps:
        c_.wait()


@jax.jit
def pallas_parallel_sum__sliding_block__moe_arch_mod__prompt_kernel(
        A_x, A_wqkv, A_wo, B_x, B_w_r, B_w_gate, B_w_up, B_w_down):
    x2 = A_x.reshape(S, D)
    wr = B_w_r.reshape(1, D)
    sc = lambda: pltpu.VMEM((HG * QB, 128), F32)
    pb = lambda: pltpu.VMEM((HG * QB, 128), BF16)
    hbm = pl.BlockSpec(memory_space=pl.ANY)
    out = pl.pallas_call(
        _kernel,
        out_shape=jax.ShapeDtypeStruct((S, D), BF16),
        in_specs=[hbm, hbm, hbm, pl.BlockSpec(memory_space=pltpu.VMEM), hbm, hbm, hbm],
        out_specs=hbm,
        scratch_shapes=[
            pltpu.VMEM((S, D), BF16),
            pltpu.VMEM((D, 3 * D), BF16),
            pltpu.VMEM((D, D), BF16),
            pltpu.VMEM((F, D), BF16),
            pltpu.VMEM((F, D), BF16),
            pltpu.VMEM((F, D), BF16),
            pltpu.VMEM((S, D), BF16),
            pltpu.SemaphoreType.DMA((2 * NCH + 6,)),
            pltpu.VMEM((S, D), BF16),
            pltpu.VMEM((NB, NG, HG * QB, 128), BF16),
            pltpu.VMEM((S + PAD, D), BF16),
            pltpu.VMEM((S + PAD, D), BF16),
            pltpu.VMEM((S, D), BF16),
            pltpu.VMEM((3, NTILE, QB, 128), F32),
            sc(), sc(), sc(), sc(), sc(), sc(),
            sc(), sc(), sc(), sc(), sc(), sc(),
            sc(), sc(), sc(), sc(),
            sc(), sc(), sc(), sc(),
            pb(), pb(), pb(), pb(), pb(), pb(),
            pb(), pb(), pb(), pb(), pb(), pb(),
        ],
        compiler_params=pltpu.CompilerParams(vmem_limit_bytes=110 * 1024 * 1024),
    )(x2, A_wqkv, A_wo, wr, B_w_gate.T, B_w_up.T, B_w_down)
    return out.reshape(1, S, D)
```

```python
import jax
import jax.numpy as jnp
from jax import lax
from jax.experimental import pallas as pl
from jax.experimental.pallas import tpu as pltpu

S, D, H, DH, WIN, F = 2048, 512, 32, 16, 256, 1376
QB = 128
NB = S // QB
HG = 128 // DH
NG = H // HG
KW = WIN + QB
NTILE = KW // 128
PAD = WIN
NEG = -1e30
LOG2E = 1.4426950408889634
CHS = (256, 256, 512, 1024)
OFFS = (0, 256, 512, 1024)
NCH = len(CHS)
LNS = 64
OCH = 4
OC = S // OCH
F32, BF16, U32 = jnp.float32, jnp.bfloat16, jnp.uint32
NT = (((1,), (1,)), ((), ()))


def _rb(t):
    return t.astype(BF16).astype(F32)


def _kernel(x_hbm, wqkv_hbm, wo_hbm, wr_ref, wg_hbm, wu_hbm, wd_hbm, o_hbm,
            x_ref, wqkv_ref, wo_ref, wg_ref, wu_ref, wd_ref, o_ref, sems,
            xn_ref, q_ref, k_ref, v_ref, att_ref, bias_ref, r_ref, y_ref, idx_ref,
            s00_ref, s01_ref, s02_ref, s10_ref, s11_ref, s12_ref,
            s20_ref, s21_ref, s22_ref, s30_ref, s31_ref, s32_ref,
            m0_ref, m1_ref, m2_ref, m3_ref, l0_ref, l1_ref, l2_ref, l3_ref,
            p00_ref, p01_ref, p02_ref, p10_ref, p11_ref, p12_ref,
            p20_ref, p21_ref, p22_ref, p30_ref, p31_ref, p32_ref):
    def cp(i, src, dst):
        return pltpu.make_async_copy(src, dst, sems.at[i])

    x_cps = [cp(c, x_hbm.at[pl.ds(OFFS[c], CHS[c])], x_ref.at[pl.ds(OFFS[c], CHS[c])])
             for c in range(NCH)]
    wq_cp = cp(NCH, wqkv_hbm.at[:, pl.ds(0, D)], wqkv_ref.at[:, pl.ds(0, D)])
    wkv_cp = cp(NCH + 1, wqkv_hbm.at[:, pl.ds(D, 2 * D)], wqkv_ref.at[:, pl.ds(D, 2 * D)])
    late_cps = [cp(NCH + 2 + i, s_, d_) for i, (s_, d_) in enumerate((
        (wg_hbm, wg_ref), (wu_hbm, wu_ref), (wd_hbm, wd_ref), (wo_hbm, wo_ref)))]
    x_cps[0].start()
    wq_cp.start()
    x_cps[0].wait()
    wq_cp.wait()
    for c_ in x_cps[1:] + [wkv_cp]:
        c_.start()

    wr = wr_ref[...].reshape(1, D).astype(F32)

    def ln_strip(r0):
        rows = slice(r0, r0 + LNS)
        x = x_ref[rows, :].astype(F32)
        mean = jnp.mean(x, axis=1, keepdims=True)
        xc = x - mean
        var = jnp.mean(xc * xc, axis=1, keepdims=True)
        d = _rb(x - _rb(mean))
        den = _rb(jnp.sqrt(_rb(_rb(var) + 1e-5)))
        xn = _rb(d / den)
        xn_ref[rows, :] = xn.astype(BF16)
        r = _rb(jnp.sum(xn * wr, axis=1, keepdims=True))
        r_ref[rows, :] = jnp.broadcast_to(r, (LNS, 128))

    for r0 in range(0, CHS[0], LNS):
        ln_strip(r0)
    for c in range(NCH):
        nxt = []
        if c + 1 < NCH:
            x_cps[c + 1].wait()
            if c + 2 == NCH:
                for c_ in late_cps:
                    c_.start()
            nxt = list(range(OFFS[c + 1], OFFS[c + 1] + CHS[c + 1], LNS))
        rows = slice(OFFS[c], OFFS[c] + CHS[c])
        per = -(-len(nxt) // NG)
        for j in range(NG):
            q = jnp.dot(xn_ref[rows, :], wqkv_ref[:, j * 128:(j + 1) * 128],
                        preferred_element_type=F32) * (DH ** -0.5 * LOG2E)
            q_ref[rows, j * 128:(j + 1) * 128] = q.astype(BF16)
            for r0 in nxt[j * per:(j + 1) * per]:
                ln_strip(r0)

    wkv_cp.wait()
    k_ref[0:PAD, :] = jnp.zeros((PAD, D), BF16)
    v_ref[0:PAD, :] = jnp.zeros((PAD, D), BF16)
    for j in range(NG):
        k_ref[PAD:, j * 128:(j + 1) * 128] = jnp.dot(
            xn_ref[...], wqkv_ref[:, D + j * 128:D + (j + 1) * 128],
            preferred_element_type=F32).astype(BF16)

    for c_ in late_cps:
        c_.wait()
    moe = {}

    def moe_piece(j):
        if j == 0:
            rsc = r_ref[...]
            rows_i = lax.broadcasted_iota(jnp.int32, (S, 128), 0)
            rmax = jnp.max(rsc)
            idx = jnp.min(jnp.where(rsc == rmax, rows_i, S))
            idx_ref[0] = idx
            base = pl.multiple_of((idx // 16) * 16, 16)
            moe["rmax"], moe["idx"], moe["base"] = rmax, idx, base
            moe["xs"] = xn_ref[pl.ds(base, 16), :]
        elif j == 1:
            moe["gp"] = _rb(lax.dot_general(moe["xs"], wg_ref[...], NT, preferred_element_type=F32))
        elif j == 2:
            up = _rb(lax.dot_general(moe["xs"], wu_ref[...], NT, preferred_element_type=F32))
            gp = moe["gp"]
            moe["h"] = (_rb(gp * _rb(jax.nn.sigmoid(gp))) * up).astype(BF16)
        else:
            y16 = _rb(jnp.dot(moe["h"], wd_ref[...], preferred_element_type=F32))
            pick = lax.broadcasted_iota(jnp.int32, (16, D), 0) == moe["idx"] - moe["base"]
            y = jnp.sum(jnp.where(pick, y16, 0.0), axis=0, keepdims=True)
            y = _rb(y * _rb(jax.nn.sigmoid(moe["rmax"])))
            y_ref[...] = jnp.broadcast_to(y, (8, D))

    for j in range(NG):
        v_ref[PAD:, j * 128:(j + 1) * 128] = jnp.dot(
            xn_ref[...], wqkv_ref[:, 2 * D + j * 128:2 * D + (j + 1) * 128],
            preferred_element_type=F32).astype(BF16)
        moe_piece(j)

    qi = lax.broadcasted_iota(jnp.int32, (QB, KW), 0)
    kj = lax.broadcasted_iota(jnp.int32, (QB, KW), 1)
    band = jnp.logical_and(qi + WIN - kj >= 0, qi + WIN - kj < WIN)
    for kind in range(3):
        ok = jnp.logical_and(band, kj >= WIN - kind * QB)
        bfull = jnp.where(ok, 0.0, NEG)
        for t in range(NTILE):
            bias_ref[kind, t] = bfull[:, t * 128:(t + 1) * 128]

    lane_head = lax.broadcasted_iota(jnp.int32, (QB, 128), 1) // DH
    s_bufs = ((s00_ref, s01_ref, s02_ref), (s10_ref, s11_ref, s12_ref),
              (s20_ref, s21_ref, s22_ref), (s30_ref, s31_ref, s32_ref))
    m_bufs, l_bufs = (m0_ref, m1_ref, m2_ref, m3_ref), (l0_ref, l1_ref, l2_ref, l3_ref)
    p_bufs = ((p00_ref, p01_ref, p02_ref), (p10_ref, p11_ref, p12_ref),
              (p20_ref, p21_ref, p22_ref), (p30_ref, p31_ref, p32_ref))
    head_masks = [jnp.where(lane_head[0:1, :] == h, jnp.uint32(0xFFFFFFFF), jnp.uint32(0))
                  for h in range(HG)]

    def masked_q(b, g):
        row0 = pl.multiple_of(b * QB, QB)
        qu = pltpu.bitcast(q_ref[pl.ds(row0, QB), g * 128:(g + 1) * 128], U32)
        return pltpu.bitcast(jnp.concatenate([qu & hm for hm in head_masks], axis=0), BF16)

    def stage_a(b, g, t, qm):
        row0 = pl.multiple_of(b * QB, QB)
        kt = k_ref[pl.ds(row0 + t * 128, 128), g * 128:(g + 1) * 128]
        s = lax.dot_general(qm, kt, NT, preferred_element_type=F32)
        bias = bias_ref[jnp.minimum(b, 2), t]
        s_bufs[g][t][...] = (s.reshape(HG, QB, 128) + bias[None]).reshape(HG * QB, 128)

    def stage_b1(g, h):
        rows = slice(h * QB, (h + 1) * QB)
        mx = jnp.maximum(jnp.maximum(s_bufs[g][0][rows, :], s_bufs[g][1][rows, :]),
                         s_bufs[g][2][rows, :])
        m = jnp.max(mx, axis=-1, keepdims=True)
        m_bufs[g][rows, :] = jnp.broadcast_to(m, (QB, 128))

    def stage_b2(g, h):
        rows = slice(h * QB, (h + 1) * QB)
        m = m_bufs[g][rows, :]
        acc = None
        for t in range(NTILE):
            pb = jnp.exp2(s_bufs[g][t][rows, :] - m).astype(BF16)
            p_bufs[g][t][rows, :] = pb
            pr = pb.astype(F32)
            acc = pr if acc is None else acc + pr
        l = jnp.sum(acc, axis=-1, keepdims=True)
        l_bufs[g][rows, :] = jnp.broadcast_to(l, (QB, 128))

    def stage_c(b, g, t, acc):
        row0 = pl.multiple_of(b * QB, QB)
        vt = v_ref[pl.ds(row0 + t * 128, 128), g * 128:(g + 1) * 128]
        r = jnp.dot(p_bufs[g][t][...], vt, preferred_element_type=F32).reshape(HG, QB, 128)
        o = r[0]
        for h in range(1, HG):
            o = jnp.where(lane_head == h, r[h], o)
        acc = o if acc is None else acc + o
        if t == NTILE - 1:
            lall = l_bufs[g][...].reshape(HG, QB, 128)
            lm = lall[0]
            for h in range(1, HG):
                lm = jnp.where(lane_head == h, lall[h], lm)
            att_ref[pl.ds(row0, QB), g * 128:(g + 1) * 128] = (acc / lm).astype(BF16)
        return acc

    def back(b, g, k):
        return (b, g - k) if g >= k else (b - 1, g - k + NG)

    def step(b, g, do_a, do_b1, do_b2, do_c):
        b1 = back(b, g, 1)
        b2 = back(b, g, 2)
        c3 = back(b, g, 3)
        heads = ((0, 1, 2), (3, 4, 5), (6, 7))
        acc = None
        qm = masked_q(b, g) if do_a else None
        for t in range(NTILE):
            if do_a:
                stage_a(b, g, t, qm)
            if do_b1:
                for h in heads[t]:
                    stage_b1(b1[1], h)
            if do_c:
                acc = stage_c(c3[0], c3[1], t, acc)
            if do_b2:
                for h in heads[t]:
                    stage_b2(b2[1], h)

    def qblock(b, first):
        for g in range(NG):
            step(b, g, True, g >= 1 or not first, g >= 2 or not first, g >= 3 or not first)

    qblock(0, True)

    def loop_body(b, carry):
        qblock(b, False)
        return carry

    lax.fori_loop(1, NB, loop_body, 0)
    step(NB, 0, False, True, True, True)
    step(NB, 1, False, False, True, True)
    step(NB, 2, False, False, False, True)

    y = y_ref[0:1, :]
    idx = idx_ref[0]
    out_cps = []
    for c in range(OCH):
        rows = slice(c * OC, (c + 1) * OC)
        sel = lax.broadcasted_iota(jnp.int32, (OC, 1), 0) + c * OC == idx
        att = _rb(jnp.dot(att_ref[rows, :], wo_ref[...], preferred_element_type=F32))
        bres = _rb(xn_ref[rows, :].astype(F32) + jnp.where(sel, y, 0.0))
        o_ref[rows, :] = (_rb(x_ref[rows, :].astype(F32) + att) + bres).astype(BF16)
        cp_out = pltpu.make_async_copy(o_ref.at[pl.ds(c * OC, OC)], o_hbm.at[pl.ds(c * OC, OC)],
                                       sems.at[NCH + 6 + c])
        cp_out.start()
        out_cps.append(cp_out)
    for c_ in out_cps:
        c_.wait()


@jax.jit
def pallas_parallel_sum__sliding_block__moe_arch_mod__prompt_kernel(
        A_x, A_wqkv, A_wo, B_x, B_w_r, B_w_gate, B_w_up, B_w_down):
    x2 = A_x.reshape(S, D)
    sc = lambda: pltpu.VMEM((HG * QB, 128), F32)
    pb = lambda: pltpu.VMEM((HG * QB, 128), BF16)
    hbm = pl.BlockSpec(memory_space=pl.ANY)
    out = pl.pallas_call(
        _kernel,
        out_shape=jax.ShapeDtypeStruct((S, D), BF16),
        in_specs=[hbm, hbm, hbm, pl.BlockSpec(memory_space=pltpu.VMEM), hbm, hbm, hbm],
        out_specs=hbm,
        scratch_shapes=[
            pltpu.VMEM((S, D), BF16),
            pltpu.VMEM((D, 3 * D), BF16),
            pltpu.VMEM((D, D), BF16),
            pltpu.VMEM((F, D), BF16),
            pltpu.VMEM((F, D), BF16),
            pltpu.VMEM((F, D), BF16),
            pltpu.VMEM((S, D), BF16),
            pltpu.SemaphoreType.DMA((NCH + 6 + OCH,)),
            pltpu.VMEM((S, D), BF16),
            pltpu.VMEM((S, D), BF16),
            pltpu.VMEM((S + PAD, D), BF16),
            pltpu.VMEM((S + PAD, D), BF16),
            pltpu.VMEM((S, D), BF16),
            pltpu.VMEM((3, NTILE, QB, 128), F32),
            pltpu.VMEM((S, 128), F32),
            pltpu.VMEM((8, D), F32),
            pltpu.SMEM((1,), jnp.int32),
            sc(), sc(), sc(), sc(), sc(), sc(),
            sc(), sc(), sc(), sc(), sc(), sc(),
            sc(), sc(), sc(), sc(),
            sc(), sc(), sc(), sc(),
            pb(), pb(), pb(), pb(), pb(), pb(),
            pb(), pb(), pb(), pb(), pb(), pb(),
        ],
        compiler_params=pltpu.CompilerParams(vmem_limit_bytes=110 * 1024 * 1024),
    )(x2, A_wqkv, A_wo, B_w_r, B_w_gate.T, B_w_up.T, B_w_down)
    return out.reshape(1, S, D)
```

```python
import jax
import jax.numpy as jnp
from jax import lax
from jax.experimental import pallas as pl
from jax.experimental.pallas import tpu as pltpu

S, D, H, DH, WIN, F = 2048, 512, 32, 16, 256, 1376
QB = 128
NB = S // QB
HG = 128 // DH
NG = H // HG
KW = WIN + QB
NTILE = KW // 128
PAD = WIN
NEG = -1e30
LOG2E = 1.4426950408889634
CHS = (256, 256, 512, 1024)
OFFS = (0, 256, 512, 1024)
NCH = len(CHS)
LNS = 64
OCH = 4
OC = S // OCH
F32, BF16, U32 = jnp.float32, jnp.bfloat16, jnp.uint32
NT = (((1,), (1,)), ((), ()))


def _rb(t):
    return t.astype(BF16).astype(F32)


def _kernel(x_hbm, wqkv_hbm, wo_hbm, wr_hbm, wg_hbm, wu_hbm, wd_hbm, o_hbm,
            x_ref, wqkv_ref, wo_ref, wr_ref, wg_ref, wu_ref, wd_ref, o_ref, sems,
            xn_ref, q_ref, k_ref, v_ref, att_ref, bias_ref, r_ref, y_ref, idx_ref,
            s00_ref, s01_ref, s02_ref, s10_ref, s11_ref, s12_ref,
            s20_ref, s21_ref, s22_ref, s30_ref, s31_ref, s32_ref,
            m0_ref, m1_ref, m2_ref, m3_ref, l0_ref, l1_ref, l2_ref, l3_ref,
            p00_ref, p01_ref, p02_ref, p10_ref, p11_ref, p12_ref,
            p20_ref, p21_ref, p22_ref, p30_ref, p31_ref, p32_ref):
    def cp(i, src, dst):
        return pltpu.make_async_copy(src, dst, sems.at[i])

    x_cps = [cp(c, x_hbm.at[pl.ds(OFFS[c], CHS[c])], x_ref.at[pl.ds(OFFS[c], CHS[c])])
             for c in range(NCH)]
    wq_cp = cp(NCH, wqkv_hbm.at[:, pl.ds(0, D)], wqkv_ref.at[:, pl.ds(0, D)])
    wkv_cp = cp(NCH + 1, wqkv_hbm.at[:, pl.ds(D, 2 * D)], wqkv_ref.at[:, pl.ds(D, 2 * D)])
    late_cps = [cp(NCH + 2 + i, s_, d_) for i, (s_, d_) in enumerate((
        (wg_hbm, wg_ref), (wu_hbm, wu_ref), (wd_hbm, wd_ref), (wo_hbm, wo_ref)))]
    wr_cp = cp(NCH + 6 + OCH, wr_hbm, wr_ref)
    x_cps[0].start()
    wq_cp.start()
    wr_cp.start()
    x_cps[0].wait()
    wq_cp.wait()
    wr_cp.wait()
    for c_ in x_cps[1:] + [wkv_cp]:
        c_.start()

    wr = wr_ref[...].reshape(1, D).astype(F32)

    def ln_strip(r0):
        rows = slice(r0, r0 + LNS)
        x = x_ref[rows, :].astype(F32)
        mean = jnp.mean(x, axis=1, keepdims=True)
        xc = x - mean
        var = jnp.mean(xc * xc, axis=1, keepdims=True)
        d = _rb(x - _rb(mean))
        den = _rb(jnp.sqrt(_rb(_rb(var) + 1e-5)))
        xn = _rb(d / den)
        xn_ref[rows, :] = xn.astype(BF16)
        r = _rb(jnp.sum(xn * wr, axis=1, keepdims=True))
        r_ref[rows, :] = jnp.broadcast_to(r, (LNS, 128))

    for r0 in range(0, CHS[0], LNS):
        ln_strip(r0)
    for c in range(NCH):
        nxt = []
        if c + 1 < NCH:
            x_cps[c + 1].wait()
            if c + 2 == NCH:
                for c_ in late_cps:
                    c_.start()
            nxt = list(range(OFFS[c + 1], OFFS[c + 1] + CHS[c + 1], LNS))
        rows = slice(OFFS[c], OFFS[c] + CHS[c])
        per = -(-len(nxt) // NG)
        for j in range(NG):
            q = jnp.dot(xn_ref[rows, :], wqkv_ref[:, j * 128:(j + 1) * 128],
                        preferred_element_type=F32) * (DH ** -0.5 * LOG2E)
            q_ref[rows, j * 128:(j + 1) * 128] = q.astype(BF16)
            for r0 in nxt[j * per:(j + 1) * per]:
                ln_strip(r0)

    wkv_cp.wait()
    k_ref[0:PAD, :] = jnp.zeros((PAD, D), BF16)
    v_ref[0:PAD, :] = jnp.zeros((PAD, D), BF16)
    for j in range(NG):
        k_ref[PAD:, j * 128:(j + 1) * 128] = jnp.dot(
            xn_ref[...], wqkv_ref[:, D + j * 128:D + (j + 1) * 128],
            preferred_element_type=F32).astype(BF16)

    for c_ in late_cps:
        c_.wait()
    moe = {}

    def moe_piece(j):
        if j == 0:
            rsc = r_ref[...]
            rows_i = lax.broadcasted_iota(jnp.int32, (S, 128), 0)
            rmax = jnp.max(rsc)
            idx = jnp.min(jnp.where(rsc == rmax, rows_i, S))
            idx_ref[0] = idx
            base = pl.multiple_of((idx // 16) * 16, 16)
            moe["rmax"], moe["idx"], moe["base"] = rmax, idx, base
            moe["xs"] = xn_ref[pl.ds(base, 16), :]
        elif j == 1:
            moe["gp"] = _rb(lax.dot_general(moe["xs"], wg_ref[...], NT, preferred_element_type=F32))
        elif j == 2:
            up = _rb(lax.dot_general(moe["xs"], wu_ref[...], NT, preferred_element_type=F32))
            gp = moe["gp"]
            moe["h"] = (_rb(gp * _rb(jax.nn.sigmoid(gp))) * up).astype(BF16)
        else:
            y16 = _rb(jnp.dot(moe["h"], wd_ref[...], preferred_element_type=F32))
            pick = lax.broadcasted_iota(jnp.int32, (16, D), 0) == moe["idx"] - moe["base"]
            y = jnp.sum(jnp.where(pick, y16, 0.0), axis=0, keepdims=True)
            y = _rb(y * _rb(jax.nn.sigmoid(moe["rmax"])))
            y_ref[...] = jnp.broadcast_to(y, (8, D))

    for j in range(NG):
        v_ref[PAD:, j * 128:(j + 1) * 128] = jnp.dot(
            xn_ref[...], wqkv_ref[:, 2 * D + j * 128:2 * D + (j + 1) * 128],
            preferred_element_type=F32).astype(BF16)
        moe_piece(j)

    qi = lax.broadcasted_iota(jnp.int32, (QB, KW), 0)
    kj = lax.broadcasted_iota(jnp.int32, (QB, KW), 1)
    band = jnp.logical_and(qi + WIN - kj >= 0, qi + WIN - kj < WIN)
    for kind in range(3):
        ok = jnp.logical_and(band, kj >= WIN - kind * QB)
        bfull = jnp.where(ok, 0.0, NEG)
        for t in range(NTILE):
            bias_ref[kind, t] = bfull[:, t * 128:(t + 1) * 128]

    lane_head = lax.broadcasted_iota(jnp.int32, (QB, 128), 1) // DH
    s_bufs = ((s00_ref, s01_ref, s02_ref), (s10_ref, s11_ref, s12_ref),
              (s20_ref, s21_ref, s22_ref), (s30_ref, s31_ref, s32_ref))
    m_bufs, l_bufs = (m0_ref, m1_ref, m2_ref, m3_ref), (l0_ref, l1_ref, l2_ref, l3_ref)
    p_bufs = ((p00_ref, p01_ref, p02_ref), (p10_ref, p11_ref, p12_ref),
              (p20_ref, p21_ref, p22_ref), (p30_ref, p31_ref, p32_ref))
    head_masks = [jnp.where(lane_head[0:1, :] == h, jnp.uint32(0xFFFFFFFF), jnp.uint32(0))
                  for h in range(HG)]

    def masked_q(b, g):
        row0 = pl.multiple_of(b * QB, QB)
        qu = pltpu.bitcast(q_ref[pl.ds(row0, QB), g * 128:(g + 1) * 128], U32)
        return pltpu.bitcast(jnp.concatenate([qu & hm for hm in head_masks], axis=0), BF16)

    def stage_a(b, g, t, qm):
        row0 = pl.multiple_of(b * QB, QB)
        kt = k_ref[pl.ds(row0 + t * 128, 128), g * 128:(g + 1) * 128]
        s = lax.dot_general(qm, kt, NT, preferred_element_type=F32)
        bias = bias_ref[jnp.minimum(b, 2), t]
        s_bufs[g][t][...] = (s.reshape(HG, QB, 128) + bias[None]).reshape(HG * QB, 128)

    def stage_b1(g, h):
        rows = slice(h * QB, (h + 1) * QB)
        mx = jnp.maximum(jnp.maximum(s_bufs[g][0][rows, :], s_bufs[g][1][rows, :]),
                         s_bufs[g][2][rows, :])
        m = jnp.max(mx, axis=-1, keepdims=True)
        m_bufs[g][rows, :] = jnp.broadcast_to(m, (QB, 128))

    def stage_b2(g, h):
        rows = slice(h * QB, (h + 1) * QB)
        m = m_bufs[g][rows, :]
        acc = None
        for t in range(NTILE):
            pb = jnp.exp2(s_bufs[g][t][rows, :] - m).astype(BF16)
            p_bufs[g][t][rows, :] = pb
            pr = pb.astype(F32)
            acc = pr if acc is None else acc + pr
        l = jnp.sum(acc, axis=-1, keepdims=True)
        l_bufs[g][rows, :] = jnp.broadcast_to(l, (QB, 128))

    def stage_c(b, g, t, acc):
        row0 = pl.multiple_of(b * QB, QB)
        vt = v_ref[pl.ds(row0 + t * 128, 128), g * 128:(g + 1) * 128]
        r = jnp.dot(p_bufs[g][t][...], vt, preferred_element_type=F32).reshape(HG, QB, 128)
        o = r[0]
        for h in range(1, HG):
            o = jnp.where(lane_head == h, r[h], o)
        acc = o if acc is None else acc + o
        if t == NTILE - 1:
            lall = l_bufs[g][...].reshape(HG, QB, 128)
            lm = lall[0]
            for h in range(1, HG):
                lm = jnp.where(lane_head == h, lall[h], lm)
            att_ref[pl.ds(row0, QB), g * 128:(g + 1) * 128] = (acc / lm).astype(BF16)
        return acc

    def back(b, g, k):
        return (b, g - k) if g >= k else (b - 1, g - k + NG)

    def step(b, g, do_a, do_b1, do_b2, do_c):
        b1 = back(b, g, 1)
        b2 = back(b, g, 2)
        c3 = back(b, g, 3)
        heads = ((0, 1, 2), (3, 4, 5), (6, 7))
        acc = None
        qm = masked_q(b, g) if do_a else None
        for t in range(NTILE):
            if do_a:
                stage_a(b, g, t, qm)
            if do_b1:
                for h in heads[t]:
                    stage_b1(b1[1], h)
            if do_c:
                acc = stage_c(c3[0], c3[1], t, acc)
            if do_b2:
                for h in heads[t]:
                    stage_b2(b2[1], h)

    def qblock(b, first):
        for g in range(NG):
            step(b, g, True, g >= 1 or not first, g >= 2 or not first, g >= 3 or not first)

    qblock(0, True)

    def loop_body(b, carry):
        qblock(b, False)
        return carry

    lax.fori_loop(1, NB, loop_body, 0)
    step(NB, 0, False, True, True, True)
    step(NB, 1, False, False, True, True)
    step(NB, 2, False, False, False, True)

    y = y_ref[0:1, :]
    idx = idx_ref[0]
    out_cps = []
    for c in range(OCH):
        rows = slice(c * OC, (c + 1) * OC)
        sel = lax.broadcasted_iota(jnp.int32, (OC, 1), 0) + c * OC == idx
        att = _rb(jnp.dot(att_ref[rows, :], wo_ref[...], preferred_element_type=F32))
        bres = _rb(xn_ref[rows, :].astype(F32) + jnp.where(sel, y, 0.0))
        o_ref[rows, :] = (_rb(x_ref[rows, :].astype(F32) + att) + bres).astype(BF16)
        cp_out = pltpu.make_async_copy(o_ref.at[pl.ds(c * OC, OC)], o_hbm.at[pl.ds(c * OC, OC)],
                                       sems.at[NCH + 6 + c])
        cp_out.start()
        out_cps.append(cp_out)
    for c_ in out_cps:
        c_.wait()


@jax.jit
def pallas_parallel_sum__sliding_block__moe_arch_mod__prompt_kernel(
        A_x, A_wqkv, A_wo, B_x, B_w_r, B_w_gate, B_w_up, B_w_down):
    x2 = A_x.reshape(S, D)
    sc = lambda: pltpu.VMEM((HG * QB, 128), F32)
    pb = lambda: pltpu.VMEM((HG * QB, 128), BF16)
    hbm = pl.BlockSpec(memory_space=pl.ANY)
    out = pl.pallas_call(
        _kernel,
        out_shape=jax.ShapeDtypeStruct((S, D), BF16),
        in_specs=[hbm, hbm, hbm, hbm, hbm, hbm, hbm],
        out_specs=hbm,
        scratch_shapes=[
            pltpu.VMEM((S, D), BF16),
            pltpu.VMEM((D, 3 * D), BF16),
            pltpu.VMEM((D, D), BF16),
            pltpu.VMEM((D,), BF16),
            pltpu.VMEM((F, D), BF16),
            pltpu.VMEM((F, D), BF16),
            pltpu.VMEM((F, D), BF16),
            pltpu.VMEM((S, D), BF16),
            pltpu.SemaphoreType.DMA((NCH + 7 + OCH,)),
            pltpu.VMEM((S, D), BF16),
            pltpu.VMEM((S, D), BF16),
            pltpu.VMEM((S + PAD, D), BF16),
            pltpu.VMEM((S + PAD, D), BF16),
            pltpu.VMEM((S, D), BF16),
            pltpu.VMEM((3, NTILE, QB, 128), F32),
            pltpu.VMEM((S, 128), F32),
            pltpu.VMEM((8, D), F32),
            pltpu.SMEM((1,), jnp.int32),
            sc(), sc(), sc(), sc(), sc(), sc(),
            sc(), sc(), sc(), sc(), sc(), sc(),
            sc(), sc(), sc(), sc(),
            sc(), sc(), sc(), sc(),
            pb(), pb(), pb(), pb(), pb(), pb(),
            pb(), pb(), pb(), pb(), pb(), pb(),
        ],
        compiler_params=pltpu.CompilerParams(vmem_limit_bytes=110 * 1024 * 1024),
    )(x2, A_wqkv, A_wo, B_w_r, B_w_gate.T, B_w_up.T, B_w_down)
    return out.reshape(1, S, D)
```
